```python
import os as _os
_os.environ.setdefault("JAX_PLATFORMS", "cpu")
import jax
import jax.numpy as jnp

def _softmax(x, axis=-1):
    return jax.nn.softmax(x, axis=axis)
def _gelu(x):
    return jax.nn.gelu(x, approximate=True)
def _silu(x):
    return jax.nn.silu(x)
def _sigmoid(x):
    return jax.nn.sigmoid(x)
def _layernorm(x, axis=-1, eps=1e-5):
    m = jnp.mean(x, axis=axis, keepdims=True)
    v = jnp.var(x, axis=axis, keepdims=True)
    return (x - m) / jnp.sqrt(v + eps)
def _scatter_add(tgt, idx, src, axis=0):
    return tgt.at[idx].add(src)
def _segment_sum(src, seg, n):
    return jax.ops.segment_sum(src, seg, n)
class _Rng:
    def __init__(self, key):
        self._k = key
    def _next(self):
        self._k, sub = jax.random.split(self._k)
        return sub
    def normal(self, shape):
        return jax.random.normal(self._next(), shape, dtype=jnp.bfloat16)
    def randint(self, lo, hi, shape):
        return jax.random.randint(self._next(), shape, lo, hi, dtype=jnp.int32)
    def uniform(self, shape, lo=0.0, hi=1.0):
        return jax.random.uniform(self._next(), shape, jnp.bfloat16, lo, hi)
    def permutation(self, n):
        return jax.random.permutation(self._next(), n)


kernel_name = 'gated_mix__ssm_conv_s5__glu_gated_geglu__prompt'

def setup_inputs():
    _rng = _Rng(jax.random.key(int.from_bytes(__import__("os").urandom(4), "little")))
    _w = (lambda a: (lambda t: t.astype(jnp.bfloat16) if jnp.issubdtype(t.dtype, jnp.floating) else t)(jnp.asarray(a)))
    def _A_setup():
        B, S, D = 1, 2048, 1024
        P = D
        Lambda_re = -0.5 * jnp.exp((lambda *s: _rng.normal(s) * 0.4)(P))
        Lambda_im = (lambda *s: _rng.normal(s) * 0.4)(P) * 1.0
        B_re = (lambda *s: _rng.normal(s) * 0.4)(P, D) * (D ** -0.5)
        B_im = (lambda *s: _rng.normal(s) * 0.4)(P, D) * (D ** -0.5)
        C_re = (lambda *s: _rng.normal(s) * 0.4)(D, P) * (P ** -0.5)
        C_im = (lambda *s: _rng.normal(s) * 0.4)(D, P) * (P ** -0.5)
        log_dt = (lambda *s: _rng.normal(s) * 0.4)(P) * 0.3 - 2.0
        Dskip = (lambda *s: _rng.normal(s) * 0.4)(D)
        return {
            "x": _w((lambda *s: _rng.normal(s) * 0.05)(B, S, D)),
            "Lambda_re": _w(Lambda_re),
            "Lambda_im": _w(Lambda_im),
            "B_re": _w(B_re),
            "B_im": _w(B_im),
            "C_re": _w(C_re),
            "C_im": _w(C_im),
            "log_dt": _w(log_dt),
            "Dskip": _w(Dskip),
        }
    _A_in = _A_setup()

    def _B_setup():
        B, S, Dm, Df = 1, 2048, 1024, 3584
        return {
            "x": _w((lambda *s: _rng.normal(s) * 0.05)(B, S, Dm)),
            "w_gate": _w((lambda *s: _rng.normal(s) * 1.6)(Dm, Df) * (Dm ** -0.5)),
            "w_up": _w((lambda *s: _rng.normal(s) * 1.6)(Dm, Df) * (Dm ** -0.5)),
            "w_down": _w((lambda *s: _rng.normal(s) * 1.6)(Df, Dm) * (Df ** -0.5)),
        }
    _B_in = _B_setup()

    return {
        "A_x": _A_in["x"],
        "A_Lambda_re": _A_in["Lambda_re"],
        "A_Lambda_im": _A_in["Lambda_im"],
        "A_B_re": _A_in["B_re"],
        "A_B_im": _A_in["B_im"],
        "A_C_re": _A_in["C_re"],
        "A_C_im": _A_in["C_im"],
        "A_log_dt": _A_in["log_dt"],
        "A_Dskip": _A_in["Dskip"],
        "B_x": _B_in["x"],
        "B_w_gate": _B_in["w_gate"],
        "B_w_up": _B_in["w_up"],
        "B_w_down": _B_in["w_down"],
        "gate_w": _w((lambda *s: _rng.normal(s) * 0.05)(1024) * 16.0),
    }

def reference(A_x, A_Lambda_re, A_Lambda_im, A_B_re, A_B_im, A_C_re, A_C_im, A_log_dt, A_Dskip, B_x, B_w_gate, B_w_up, B_w_down, gate_w):
    def _A_ref(x, Lambda_re, Lambda_im, B_re, B_im, C_re, C_im, log_dt, Dskip):
        Bsz, L, H = x.shape
        Lam = Lambda_re + 1j * Lambda_im
        Bmat = B_re + 1j * B_im
        Cmat = C_re + 1j * C_im
        dt = jnp.exp(log_dt)
        Lam_bar = jnp.exp(dt * Lam)
        B_bar = ((Lam_bar - 1.0) / Lam)[:, None] * Bmat
        Bu = jnp.einsum("bld,pd->blp", x + 0j, B_bar)
        h = jnp.zeros_like(Bu[:, 0, :])
        hs = []
        for t in range(L):
            h = Lam_bar[None, :] * h + Bu[:, t, :]
            hs.append(h)
        hseq = jnp.stack(hs, 1)
        y = 2.0 * jnp.einsum("blp,dp->bld", hseq, Cmat).real + x * Dskip[None, None, :]
        return y

    def _B_ref(x, w_gate, w_up, w_down):
        g = jnp.einsum("bsd,df->bsf", x, w_gate)
        u = jnp.einsum("bsd,df->bsf", x, w_up)
        h = _gelu(g) * u
        return jnp.einsum("bsf,fd->bsd", h, w_down)

    x = A_x
    g = _sigmoid((x * gate_w).sum(-1, keepdims=True))
    a = _A_ref(x, A_Lambda_re, A_Lambda_im, A_B_re, A_B_im, A_C_re, A_C_im, A_log_dt, A_Dskip)
    b = _B_ref(x, B_w_gate, B_w_up, B_w_down)
    return g * a + (1 - g) * b
```

```python
import jax
import jax.numpy as jnp
from jax import lax
import jax.experimental.pallas as pl
import jax.experimental.pallas.tpu as pltpu

F32 = jnp.float32
BF16 = jnp.bfloat16
U32 = jnp.uint32
NN = (((1,), (0,)), ((), ()))
NT = (((1,), (1,)), ((), ()))

A_FORM = [((1, 0), (1, 3)), ((1, 2), (1, 3)), ((1, 0),), ((1, 3),), ((1, 0), (1, 1)), ((1, 2), (-1, 0)), ((1, 1), (-1, 3))]
B_FORM = [((1, 0), (1, 3)), ((1, 0),), ((1, 1), (-1, 3)), ((1, 2), (-1, 0)), ((1, 3),), ((1, 0), (1, 1)), ((1, 2), (1, 3))]
C_FORM = [((1, 0), (1, 3), (-1, 4), (1, 6)), ((1, 2), (1, 4)), ((1, 1), (1, 3)), ((1, 0), (-1, 1), (1, 2), (1, 5))]

TF = 512
G = 128
RX = 256
RO = 64
NCONST = 14


def _dot(a, b, dn=NN):
    return lax.dot_general(a, b, dn, preferred_element_type=F32)


class _Pair:
    def __init__(self, lo, hi):
        self.lo, self.hi = lo, hi

    def __add__(self, o):
        return _Pair(self.lo + o.lo, self.hi + o.hi)

    def __sub__(self, o):
        return _Pair(self.lo - o.lo, self.hi - o.hi)

    def pack(self):
        return pltpu.pack_elementwise([self.lo, self.hi], packed_dtype=BF16)


def _split(tile):
    w = pltpu.bitcast(tile, U32)
    return _Pair(pltpu.unpack_elementwise(w, index=0, packed_dtype=BF16, unpacked_dtype=F32),
                 pltpu.unpack_elementwise(w, index=1, packed_dtype=BF16, unpacked_dtype=F32))


def _as_bf16(words):
    return pltpu.bitcast(words, BF16)


def _lin(form, get):
    out = None
    for sgn, idx in form:
        t = get(idx)
        out = t if out is None else (out + t if sgn > 0 else out - t)
    return out


class _Side:
    def __init__(self, raw, lvl, form):
        self.raw, self.lvl, self.form, self.memo = raw, lvl, form, {}

    def node(self, path, i, j):
        key = (path, i, j)
        if key not in self.memo:
            if not path:
                self.memo[key] = self.raw(i, j)
            else:
                n = 2 ** (self.lvl - len(path))
                self.memo[key] = _lin(self.form[path[-1]],
                                      lambda q: self.node(path[:-1], (q // 2) * n + i, (q % 2) * n + j))
        return self.memo[key]

    def leaf(self, path):
        return self.node(tuple(path), 0, 0)


class _Out:
    def __init__(self, prod, lvl):
        self.prod, self.lvl, self.memo = prod, lvl, {}

    def node(self, path, i, j):
        key = (path, i, j)
        if key not in self.memo:
            if len(path) == self.lvl:
                self.memo[key] = self.prod(path)
            else:
                n = 2 ** (self.lvl - len(path) - 1)
                self.memo[key] = _lin(C_FORM[(i // n) * 2 + (j // n)],
                                      lambda m: self.node(path + (m,), i % n, j % n))
        return self.memo[key]

    def block(self, i, j):
        return self.node((), i, j)


PATHS2 = [(i, j) for i in range(7) for j in range(7)]


def _is_raw(path):
    return all(len(A_FORM[a]) == 1 for a in path)


def _raw_pos(path):
    i = j = 0
    for a in path:
        q = A_FORM[a][0][1]
        i, j = 2 * i + q // 2, 2 * j + q % 2
    return i, j


def _cmul(ar, ai, br, bi):
    return ar * br - ai * bi, ar * bi + ai * br


def _cdiv(ar, ai, br, bi):
    big = jnp.abs(br) >= jnp.abs(bi)
    p = jnp.where(big, bi, br)
    q = jnp.where(big, br, bi)
    r = p / q
    den = q + p * r
    u = jnp.where(big, ar, ai)
    v = jnp.where(big, ai, ar)
    re = (u + v * r) / den
    im = (v - u * r) / den
    return re, jnp.where(big, im, -im)


def _setup_consts(lre_ref, lim_ref, ldt_ref, cst):
    P = lre_ref.shape[0]

    def ld(r):
        return jnp.broadcast_to(r[...].astype(F32).reshape(1, P), (8, P))

    lre, lim, ldt = ld(lre_ref), ld(lim_ref), ld(ldt_ref)
    dt = jnp.exp(ldt).astype(ldt_ref.dtype).astype(F32)
    s = lax.broadcasted_iota(jnp.int32, (8, P), 0)
    k = (s + 1).astype(F32)
    zr = dt * lre
    zi = dt * lim
    mag = jnp.exp(zr * k)
    pr = mag * jnp.cos(zi * k)
    pi = mag * jnp.sin(zi * k)

    def row(a, r):
        return jnp.broadcast_to(a[r:r + 1, :], (8, P))

    cr, ci = _cdiv(row(pr, 0) - 1.0, row(pi, 0), lre, lim)
    vals = [jnp.where(s == 0, row(pr, 0), 0.0), jnp.where(s == 0, row(pi, 0), 0.0), 2.0 * cr, 2.0 * ci]
    for kk in (1, 2, 4):
        vals.append(jnp.where(s >= kk, row(pr, kk - 1), 0.0))
        vals.append(jnp.where(s >= kk, row(pi, kk - 1), 0.0))
    vals += [pr, pi, row(pr, 7), row(pi, 7)]
    for i, v in enumerate(vals):
        for c in range(P // G):
            cst[c, i] = v[:, c * G:(c + 1) * G]


class _Scan:
    def __init__(self, vr_fn, vi_fn, cst, g_fn, store):
        self.vr_fn, self.vi_fn, self.g_fn, self.store = vr_fn, vi_fn, g_fn, store
        self.k = [cst[i] for i in range(NCONST)]
        self.c = None

    def _prefix(self, vr, vi):
        k = self.k
        for a, kk in enumerate((1, 2, 4)):
            tr, ti = _cmul(k[4 + 2 * a], k[5 + 2 * a], pltpu.roll(vr, kk, 0), pltpu.roll(vi, kk, 0))
            vr, vi = vr + tr, vi + ti
        return vr, vi

    def _finish(self, zs, j0, j1):
        k = self.k
        gs_all = self.g_fn(j0 * 8, j1 * 8)
        hr, hi = [], []
        for j, (zr, zi) in enumerate(zs):
            gs = gs_all[j * 8:(j + 1) * 8]
            zr, zi = zr * gs, zi * gs
            hr.append(k[2] * zr - k[3] * zi)
            hi.append(-(k[2] * zi + k[3] * zr))
        self.store(j0 * 8, j1 * 8, jnp.concatenate(hr, 0).astype(BF16), jnp.concatenate(hi, 0).astype(BF16))

    def piece(self, j0, j1):
        k = self.k
        vr_all, vi_all = self.vr_fn(j0 * 8, j1 * 8), self.vi_fn(j0 * 8, j1 * 8)
        zs = []
        for j in range(j1 - j0):
            vr, vi = vr_all[j * 8:(j + 1) * 8], vi_all[j * 8:(j + 1) * 8]
            if self.c is not None:
                tr, ti = _cmul(k[0], k[1], pltpu.roll(self.c[0], 1, 0), pltpu.roll(self.c[1], 1, 0))
                vr, vi = vr + tr, vi + ti
            self.c = self._prefix(vr, vi)
            zs.append(self.c)
        self._finish(zs, j0, j1)

    def piece_parallel(self, j0, j1):
        k = self.k
        vr_all, vi_all = self.vr_fn(j0 * 8, j1 * 8), self.vi_fn(j0 * 8, j1 * 8)
        zs = []
        for j in range(j1 - j0):
            vr, vi = self._prefix(vr_all[j * 8:(j + 1) * 8], vi_all[j * 8:(j + 1) * 8])
            cr, ci = self.c
            tr, ti = _cmul(k[10], k[11], cr, ci)
            zs.append((vr + tr, vi + ti))
            tr, ti = _cmul(k[12], k[13], cr, ci)
            self.c = (tr + jnp.broadcast_to(vr[7:8, :], (8, G)), ti + jnp.broadcast_to(vi[7:8, :], (8, G)))
        self._finish(zs, j0, j1)


def _gelu_glu(gate, up, half_scale):
    inner = gate * (0.7978845608028654 + (0.7978845608028654 * 0.044715) * (gate * gate))
    a = gate * (up * half_scale)
    return a + a * jnp.tanh(inner)


def _make_kernel(S, D, P, F):
    NF = F // TF
    Q = S // 4
    KQ = D // 4
    ND = D // 4
    KO = P // 2
    NX = S // RX
    NO = Q // RO
    R = 16

    def kernel(lre_ref, lim_ref, ldt_ref, dsk_ref, gw_ref,
               x_h, bre_h, bim_h, cre_h, cim_h, wg_h, wu_h, wd_h, out_h,
               x_v, xa1, xa2, acc, hre, him, wg_v, wu_v, wd_v, bre_v, bim_v, cre_v, cim_v, cc,
               b0w, va, vb, gb, cst, carry, ost, sem_x, sem_b, sem_w, sem_c, sem_o):

        def w_copies(f, slot):
            cs = pl.ds(pl.multiple_of(f * TF, TF), TF)
            rs = pl.ds(pl.multiple_of((f + 1) * G, G), G)
            return [
                pltpu.make_async_copy(bre_h.at[rs, :], bre_v.at[slot], sem_w.at[slot * 5 + 0]),
                pltpu.make_async_copy(bim_h.at[rs, :], bim_v.at[slot], sem_w.at[slot * 5 + 1]),
                pltpu.make_async_copy(wg_h.at[:, cs], wg_v.at[slot], sem_w.at[slot * 5 + 2]),
                pltpu.make_async_copy(wu_h.at[:, cs], wu_v.at[slot], sem_w.at[slot * 5 + 3]),
                pltpu.make_async_copy(wd_h.at[cs, :], wd_v.at[slot], sem_w.at[slot * 5 + 4]),
            ]

        def row0(n, size):
            return n * size if isinstance(n, int) else pl.multiple_of(n * size, size)

        def x_copy(n):
            r0 = row0(n, RX)
            return pltpu.make_async_copy(x_h.at[0, pl.ds(r0, RX), :], x_v.at[pl.ds(r0, RX), :], sem_x.at[n % 2])

        cb0r = pltpu.make_async_copy(bre_h.at[0:G, :], bre_v.at[1], sem_b.at[0])
        cb0i = pltpu.make_async_copy(bim_h.at[0:G, :], bim_v.at[1], sem_b.at[1])
        cb0r.start()
        cb0i.start()
        x_copy(0).start()
        x_copy(1).start()
        _setup_consts(lre_ref, lim_ref, ldt_ref, cst)
        carry[...] = jnp.zeros_like(carry)
        cb0r.wait()
        cb0i.wait()
        b0w[0] = pltpu.bitcast(bre_v[1], U32)
        b0w[1] = pltpu.bitcast(bim_v[1], U32)
        gw = gw_ref[...].astype(F32).reshape(1, D)

        def x_wait_start(n):
            x_copy(n).wait()

            @pl.when(n + 2 < NX)
            def _():
                x_copy(n + 2).start()

            @pl.when(n == NX - 3)
            def _():
                for c in w_copies(0, 0):
                    c.start()

        def gate_rows(n):
            r0 = row0(n, RX)
            for rt in range(RX // 8):
                rows = pl.ds(r0 + rt * 8, 8)
                t = None
                for lt in range(D // 128):
                    ls = slice(lt * 128, (lt + 1) * 128)
                    p = x_v[rows, ls].astype(F32) * gw[:, ls]
                    t = p if t is None else t + p
                g = jax.nn.sigmoid(jnp.sum(t, axis=-1, keepdims=True))
                gb[rows, :] = jnp.broadcast_to(g, (8, 128))

        def in_proj0(n, vbuf):
            lhs = x_v[pl.ds(row0(n, RX), RX), :]
            for ri in range(2):
                vbuf[ri] = _dot(lhs, _as_bf16(b0w[ri]), NT)

        def scan0(n, vbuf, parallel=False):
            r0 = row0(n, RX)

            def store(a, b, hr, hi):
                hre[pl.ds(r0 + a, b - a), 0:G] = hr
                him[pl.ds(r0 + a, b - a), 0:G] = hi

            sc = _Scan(lambda a, b: vbuf[0, a:b, :], lambda a, b: vbuf[1, a:b, :], cst.at[0],
                       lambda a, b: gb[pl.ds(r0 + a, b - a), :], store)
            cr, ci = carry[0], carry[1]
            if parallel:
                sc.c = (jnp.broadcast_to(cr[7:8, :], (8, G)), jnp.broadcast_to(ci[7:8, :], (8, G)))
                sc.piece_parallel(0, RX // 8)
            else:
                sc.c = (cr, ci)
                for j in range(0, RX // 8, 8):
                    sc.piece(j, j + 8)
                carry[0] = sc.c[0]
                carry[1] = sc.c[1]

        def pro_body(m, _):
            x_wait_start(2 * m + 1)
            in_proj0(2 * m + 1, vb)
            scan0(2 * m, va)
            gate_rows(2 * m + 1)
            x_wait_start(2 * m + 2)
            in_proj0(2 * m + 2, va)
            scan0(2 * m + 1, vb)
            gate_rows(2 * m + 2)
            return 0

        x_wait_start(0)
        in_proj0(0, va)
        gate_rows(0)
        lax.fori_loop(0, NX // 2 - 1, pro_body, 0)
        x_wait_start(NX - 1)
        in_proj0(NX - 1, vb)
        scan0(NX - 2, va)
        gate_rows(NX - 1)
        scan0(NX - 1, vb, parallel=True)

        def xc2_body(n, _):
            r0, r0h = row0(n, 16), row0(n, 8)
            for lt in range(KQ // 128):
                def raw_x(q, k):
                    c0 = k * KQ + lt * 128
                    return _split(x_v[pl.ds(q * Q + r0, 16), c0:c0 + 128])
                sd = _Side(raw_x, 2, A_FORM)
                for p in PATHS2:
                    if not _is_raw(p):
                        xa2[7 * p[0] + p[1], pl.ds(r0h, 8), lt * 128:(lt + 1) * 128] = sd.leaf(p).pack()
            return 0

        def xc1_body(n, _):
            r0, r0h = row0(n, 32), row0(n, 16)
            for rt in range(2):
                for lt in range(D // 2 // 128):
                    def raw_x(hf, k):
                        c0 = k * (D // 2) + lt * 128
                        return _split(x_v[pl.ds(hf * 2 * Q + r0 + rt * 16, 16), c0:c0 + 128])
                    sd = _Side(raw_x, 1, A_FORM)
                    for i in range(7):
                        if not _is_raw((i,)):
                            xa1[i, pl.ds(r0h + rt * 8, 8), lt * 128:(lt + 1) * 128] = sd.leaf((i,)).pack()
            return 0

        lax.fori_loop(0, Q // 16, xc2_body, 0)
        lax.fori_loop(0, 2 * Q // 32, xc1_body, 0)

        def xa1_op(i):
            if not _is_raw((i,)):
                return _as_bf16(xa1[i])
            a, b = _raw_pos((i,))
            return x_v[a * 2 * Q:(a + 1) * 2 * Q, b * 2 * KQ:(b + 1) * 2 * KQ]

        def xa2_op(p):
            if not _is_raw(p):
                return _as_bf16(xa2[7 * p[0] + p[1]])
            a, b = _raw_pos(p)
            return x_v[a * Q:(a + 1) * Q, b * KQ:(b + 1) * KQ]

        ccr = pltpu.make_async_copy(cre_h, cre_v, sem_c.at[0])
        cci = pltpu.make_async_copy(cim_h, cim_v, sem_c.at[1])

        def body(f, _):
            slot = f % 2

            @pl.when(f < NF - 1)
            def _():
                for c in w_copies(f + 1, 1 - slot):
                    c.start()

            @pl.when(f == NF - 1)
            def _():
                ccr.start()
                cci.start()

            for c in w_copies(f, slot):
                c.wait()

            K2 = D // 2

            def raw_b(i, j):
                src = bre_v if j == 0 else bim_v
                return src[slot, :, i * K2:(i + 1) * K2].astype(F32)

            sb = _Side(raw_b, 1, B_FORM)
            ipp = {(i,): _dot(xa1_op(i), sb.leaf((i,)).astype(BF16), NT) for i in (4, 0, 2, 3, 6, 1, 5)}
            v = _Out(lambda p: ipp[p], 1)

            NQ = TF // 2

            def raw_w(i, j):
                src = wg_v if j < 2 else wu_v
                return src[slot, i * KQ:(i + 1) * KQ, (j % 2) * NQ:(j % 2 + 1) * NQ].astype(F32)

            sw = _Side(raw_w, 2, B_FORM)
            gu = {}
            outs = [_Out((lambda p, t=t: gu[p][t * R:(t + 1) * R]), 2) for t in range(Q // R)]
            for i in range(7):
                for j in range(7):
                    gu[(i, j)] = _dot(xa2_op((i, j)), sw.leaf((i, j)).astype(BF16))
                for o in outs:
                    for a in range(2):
                        for b in range(2):
                            o.node((i,), a, b)

            h = {}
            for t, o in enumerate(outs):
                for q in range(4):
                    hs = 0.5 - 0.5 * gb[q * Q + t * R:q * Q + (t + 1) * R, :]
                    hs = jnp.concatenate([hs, hs], 1)
                    for j in range(2):
                        hq = _gelu_glu(o.block(q, j), o.block(q, 2 + j), hs)
                        for l in range(2):
                            h[(q, 2 * j + l, t)] = hq[:, l * 128:(l + 1) * 128]

            H = S // 2
            cs = pl.ds(pl.multiple_of((f + 1) * G, G), G)

            def v_rows(ri):
                return lambda a, b: (v.block(0, ri)[a:b] if b <= H else v.block(1, ri)[a - H:b - H])

            def store(a, b, hr, hi):
                hre[a:b, cs] = hr
                him[a:b, cs] = hi

            sc = _Scan(v_rows(0), v_rows(1), cst.at[f + 1], lambda a, b: gb[a:b, :], store)
            for j in range(0, S // 8, 8):
                sc.piece(j, j + 8)

            KD = TF // 4
            sides = [_Side((lambda q, k, t=t: h[(q, k, t)]), 2, A_FORM) for t in range(Q // R)]

            def raw_d(i, j):
                return wd_v[slot, i * KD:(i + 1) * KD, j * ND:(j + 1) * ND].astype(F32)

            sdn = _Side(raw_d, 2, B_FORM)
            for p in PATHS2:
                lhs = jnp.concatenate([sd.leaf(p) for sd in sides], 0).astype(BF16)
                m = _dot(lhs, sdn.leaf(p).astype(BF16))
                acc[7 * p[0] + p[1]] = jnp.where(f > 0, acc[7 * p[0] + p[1]], 0.0) + m
            return 0

        lax.fori_loop(0, NF, body, 0)

        ccr.wait()
        cci.wait()

        def cc_body(n, _):
            r0, r0h = row0(n, 16), row0(n, 8)
            for lt in range(KO // 128):
                def raw_c(k, nq):
                    src = cre_v if k < 2 else cim_v
                    c0 = (k % 2) * KO + lt * 128
                    return _split(src[pl.ds(nq * ND + r0, 16), c0:c0 + 128])
                sd = _Side(raw_c, 2, B_FORM)
                for p in PATHS2:
                    cc[7 * p[0] + p[1], pl.ds(r0h, 8), lt * 128:(lt + 1) * 128] = sd.leaf(p).pack()
            return 0

        lax.fori_loop(0, ND // 16, cc_body, 0)

        dsk = dsk_ref[...].astype(F32).reshape(1, D)
        order = (2, 3, 1, 4, 0, 5, 6)

        def o_copies(r, slot):
            r0 = row0(r, RO)
            return [pltpu.make_async_copy(ost.at[slot, q], out_h.at[0, pl.ds(q * Q + r0, RO), :],
                                          sem_o.at[slot * 4 + q]) for q in range(4)]

        def obody(r, _):
            slot = r % 2
            r0 = row0(r, RO)

            @pl.when(r >= 2)
            def _():
                for c in o_copies(r - 2, slot):
                    c.wait()

            def h_block(q, k):
                src = hre if k < 2 else him
                return src[pl.ds(q * Q + r0, RO), (k % 2) * KO:(k % 2 + 1) * KO]

            sh = _Side(lambda q, k: _split(h_block(q, k)), 2, A_FORM)
            tot = {}
            for i in order:
                for j in order:
                    p = (i, j)
                    lhs = h_block(*_raw_pos(p)) if _is_raw(p) else _as_bf16(sh.leaf(p).pack())
                    tot[p] = acc[7 * i + j, pl.ds(r0, RO), :] + _dot(lhs, _as_bf16(cc[7 * i + j]), NT)
            for rt in range(RO // 8):
                for lt in range(ND // 128):
                    o = _Out(lambda p: tot[p][rt * 8:(rt + 1) * 8, lt * 128:(lt + 1) * 128], 2)
                    for q in range(4):
                        rows = pl.ds(q * Q + r0 + rt * 8, 8)
                        gq = gb[rows, :]
                        for nq in range(4):
                            c0 = nq * ND + lt * 128
                            skip = x_v[rows, c0:c0 + 128].astype(F32) * dsk[:, c0:c0 + 128]
                            ost[slot, q, rt * 8:(rt + 1) * 8, c0:c0 + 128] = o.block(q, nq) + skip * gq
            for c in o_copies(r, slot):
                c.start()
            return 0

        lax.fori_loop(0, NO, obody, 0)
        for r in (NO - 2, NO - 1):
            for c in o_copies(r, r % 2):
                c.wait()

    return kernel


@jax.jit
def pallas_gated_mix__ssm_conv_s5__glu_gated_geglu__prompt_kernel(
    A_x: jax.Array,
    A_Lambda_re: jax.Array,
    A_Lambda_im: jax.Array,
    A_B_re: jax.Array,
    A_B_im: jax.Array,
    A_C_re: jax.Array,
    A_C_im: jax.Array,
    A_log_dt: jax.Array,
    A_Dskip: jax.Array,
    B_x: jax.Array,
    B_w_gate: jax.Array,
    B_w_up: jax.Array,
    B_w_down: jax.Array,
    gate_w: jax.Array,
):
    del B_x
    nb, S, D = A_x.shape
    P = A_Lambda_re.shape[0]
    F = B_w_gate.shape[1]
    assert nb == 1 and P == D and P // G == F // TF + 1 and F % TF == 0
    assert D % 1024 == 0 and S % 2048 == 0 and (S // RX) % 2 == 0 and S // RX >= 4
    Q = S // 4

    vmem = pl.BlockSpec(memory_space=pltpu.VMEM)
    hbm = pl.BlockSpec(memory_space=pl.ANY)
    return pl.pallas_call(
        _make_kernel(S, D, P, F),
        in_specs=[vmem] * 5 + [hbm] * 8,
        out_specs=hbm,
        out_shape=jax.ShapeDtypeStruct((1, S, D), F32),
        scratch_shapes=[
            pltpu.VMEM((S, D), BF16),
            pltpu.VMEM((7, S // 4, D // 2), U32),
            pltpu.VMEM((49, Q // 2, D // 4), U32),
            pltpu.VMEM((49, Q, D // 4), F32),
            pltpu.VMEM((S, P), BF16),
            pltpu.VMEM((S, P), BF16),
            pltpu.VMEM((2, D, TF), BF16),
            pltpu.VMEM((2, D, TF), BF16),
            pltpu.VMEM((2, TF, D), BF16),
            pltpu.VMEM((2, G, D), BF16),
            pltpu.VMEM((2, G, D), BF16),
            pltpu.VMEM((D, P), BF16),
            pltpu.VMEM((D, P), BF16),
            pltpu.VMEM((49, D // 8, P // 2), U32),
            pltpu.VMEM((2, G // 2, D), U32),
            pltpu.VMEM((2, RX, G), F32),
            pltpu.VMEM((2, RX, G), F32),
            pltpu.VMEM((S, 128), F32),
            pltpu.VMEM((P // G, NCONST, 8, G), F32),
            pltpu.VMEM((2, 8, G), F32),
            pltpu.VMEM((2, 4, RO, D), F32),
            pltpu.SemaphoreType.DMA((2,)),
            pltpu.SemaphoreType.DMA((2,)),
            pltpu.SemaphoreType.DMA((10,)),
            pltpu.SemaphoreType.DMA((2,)),
            pltpu.SemaphoreType.DMA((8,)),
        ],
        compiler_params=pltpu.CompilerParams(vmem_limit_bytes=126 * 1024 * 1024),
    )(A_Lambda_re, A_Lambda_im, A_log_dt, A_Dskip, gate_w,
      A_x, A_B_re, A_B_im, A_C_re, A_C_im, B_w_gate, B_w_up, B_w_down)
```

```python
import jax
import jax.numpy as jnp
from jax import lax
import jax.experimental.pallas as pl
import jax.experimental.pallas.tpu as pltpu

F32 = jnp.float32
BF16 = jnp.bfloat16
U32 = jnp.uint32
NN = (((1,), (0,)), ((), ()))
NT = (((1,), (1,)), ((), ()))

A_FORM = [((1, 0), (1, 3)), ((1, 2), (1, 3)), ((1, 0),), ((1, 3),), ((1, 0), (1, 1)), ((1, 2), (-1, 0)), ((1, 1), (-1, 3))]
B_FORM = [((1, 0), (1, 3)), ((1, 0),), ((1, 1), (-1, 3)), ((1, 2), (-1, 0)), ((1, 3),), ((1, 0), (1, 1)), ((1, 2), (1, 3))]
C_FORM = [((1, 0), (1, 3), (-1, 4), (1, 6)), ((1, 2), (1, 4)), ((1, 1), (1, 3)), ((1, 0), (-1, 1), (1, 2), (1, 5))]

TF = 512
G = 128
RX = 256
RO = 64
NCONST = 14

IP_ORDER = (1, 0, 6, 3, 4, 2, 5)
GU_ORDER = ((2, 0, 5, 1, 3, 4, 6), (1, 0, 3, 4, 2, 5, 6))
DN_ORDER = ((0, 6, 2, 4, 1, 3, 5), (4, 6, 3, 1, 0, 5, 2))
OP_ORDER = ((2, 3, 4, 1, 0, 5, 6), (2, 3, 5, 4, 1, 0, 6))
SCAN_AFTER = (2, 6)


def _dot(a, b, dn=NN):
    return lax.dot_general(a, b, dn, preferred_element_type=F32)


class _Pair:
    def __init__(self, lo, hi):
        self.lo, self.hi = lo, hi

    def __add__(self, o):
        return _Pair(self.lo + o.lo, self.hi + o.hi)

    def __sub__(self, o):
        return _Pair(self.lo - o.lo, self.hi - o.hi)

    def pack(self):
        return pltpu.pack_elementwise([self.lo, self.hi], packed_dtype=BF16)


def _split(tile):
    w = pltpu.bitcast(tile, U32)
    return _Pair(pltpu.unpack_elementwise(w, index=0, packed_dtype=BF16, unpacked_dtype=F32),
                 pltpu.unpack_elementwise(w, index=1, packed_dtype=BF16, unpacked_dtype=F32))


def _as_bf16(words):
    return pltpu.bitcast(words, BF16)


def _lin(form, get):
    out = None
    for sgn, idx in form:
        t = get(idx)
        out = t if out is None else (out + t if sgn > 0 else out - t)
    return out


class _Side:
    def __init__(self, raw, lvl, form):
        self.raw, self.lvl, self.form, self.memo = raw, lvl, form, {}

    def node(self, path, i, j):
        key = (path, i, j)
        if key not in self.memo:
            if not path:
                self.memo[key] = self.raw(i, j)
            else:
                n = 2 ** (self.lvl - len(path))
                self.memo[key] = _lin(self.form[path[-1]],
                                      lambda q: self.node(path[:-1], (q // 2) * n + i, (q % 2) * n + j))
        return self.memo[key]

    def leaf(self, path):
        return self.node(tuple(path), 0, 0)


class _Out:
    def __init__(self, prod, lvl):
        self.prod, self.lvl, self.memo = prod, lvl, {}

    def node(self, path, i, j):
        key = (path, i, j)
        if key not in self.memo:
            if len(path) == self.lvl:
                self.memo[key] = self.prod(path)
            else:
                n = 2 ** (self.lvl - len(path) - 1)
                self.memo[key] = _lin(C_FORM[(i // n) * 2 + (j // n)],
                                      lambda m: self.node(path + (m,), i % n, j % n))
        return self.memo[key]

    def block(self, i, j):
        return self.node((), i, j)


PATHS2 = [(i, j) for i in range(7) for j in range(7)]


def _is_raw(path):
    return all(len(A_FORM[a]) == 1 for a in path)


def _raw_pos(path):
    i = j = 0
    for a in path:
        q = A_FORM[a][0][1]
        i, j = 2 * i + q // 2, 2 * j + q % 2
    return i, j


def _cmul(ar, ai, br, bi):
    return ar * br - ai * bi, ar * bi + ai * br


def _cdiv(ar, ai, br, bi):
    big = jnp.abs(br) >= jnp.abs(bi)
    p = jnp.where(big, bi, br)
    q = jnp.where(big, br, bi)
    r = p / q
    den = q + p * r
    u = jnp.where(big, ar, ai)
    v = jnp.where(big, ai, ar)
    re = (u + v * r) / den
    im = (v - u * r) / den
    return re, jnp.where(big, im, -im)


def _setup_consts(lre_ref, lim_ref, ldt_ref, cst):
    P = lre_ref.shape[0]

    def ld(r):
        return jnp.broadcast_to(r[...].astype(F32).reshape(1, P), (8, P))

    lre, lim, ldt = ld(lre_ref), ld(lim_ref), ld(ldt_ref)
    dt = jnp.exp(ldt).astype(ldt_ref.dtype).astype(F32)
    s = lax.broadcasted_iota(jnp.int32, (8, P), 0)
    k = (s + 1).astype(F32)
    zr = dt * lre
    zi = dt * lim
    mag = jnp.exp(zr * k)
    pr = mag * jnp.cos(zi * k)
    pi = mag * jnp.sin(zi * k)

    def row(a, r):
        return jnp.broadcast_to(a[r:r + 1, :], (8, P))

    cr, ci = _cdiv(row(pr, 0) - 1.0, row(pi, 0), lre, lim)
    vals = [jnp.where(s == 0, row(pr, 0), 0.0), jnp.where(s == 0, row(pi, 0), 0.0), 2.0 * cr, 2.0 * ci]
    for kk in (1, 2, 4):
        vals.append(jnp.where(s >= kk, row(pr, kk - 1), 0.0))
        vals.append(jnp.where(s >= kk, row(pi, kk - 1), 0.0))
    vals += [pr, pi, row(pr, 7), row(pi, 7)]
    for i, v in enumerate(vals):
        for c in range(P // G):
            cst[c, i] = v[:, c * G:(c + 1) * G]


class _Scan:
    def __init__(self, vr_fn, vi_fn, cst, g_fn, store):
        self.vr_fn, self.vi_fn, self.g_fn, self.store = vr_fn, vi_fn, g_fn, store
        self.k = [cst[i] for i in range(NCONST)]
        self.c = None

    def _prefix(self, vr, vi):
        k = self.k
        for a, kk in enumerate((1, 2, 4)):
            tr, ti = _cmul(k[4 + 2 * a], k[5 + 2 * a], pltpu.roll(vr, kk, 0), pltpu.roll(vi, kk, 0))
            vr, vi = vr + tr, vi + ti
        return vr, vi

    def _finish(self, zs, j0, j1):
        k = self.k
        gs_all = self.g_fn(j0 * 8, j1 * 8)
        hr, hi = [], []
        for j, (zr, zi) in enumerate(zs):
            gs = gs_all[j * 8:(j + 1) * 8]
            zr, zi = zr * gs, zi * gs
            hr.append(k[2] * zr - k[3] * zi)
            hi.append(-(k[2] * zi + k[3] * zr))
        self.store(j0 * 8, j1 * 8, jnp.concatenate(hr, 0).astype(BF16), jnp.concatenate(hi, 0).astype(BF16))

    def piece(self, j0, j1):
        k = self.k
        vr_all, vi_all = self.vr_fn(j0 * 8, j1 * 8), self.vi_fn(j0 * 8, j1 * 8)
        zs = []
        for j in range(j1 - j0):
            vr, vi = vr_all[j * 8:(j + 1) * 8], vi_all[j * 8:(j + 1) * 8]
            if self.c is not None:
                tr, ti = _cmul(k[0], k[1], pltpu.roll(self.c[0], 1, 0), pltpu.roll(self.c[1], 1, 0))
                vr, vi = vr + tr, vi + ti
            self.c = self._prefix(vr, vi)
            zs.append(self.c)
        self._finish(zs, j0, j1)

    def piece_parallel(self, j0, j1):
        k = self.k
        vr_all, vi_all = self.vr_fn(j0 * 8, j1 * 8), self.vi_fn(j0 * 8, j1 * 8)
        zs = []
        for j in range(j1 - j0):
            vr, vi = self._prefix(vr_all[j * 8:(j + 1) * 8], vi_all[j * 8:(j + 1) * 8])
            cr, ci = self.c
            tr, ti = _cmul(k[10], k[11], cr, ci)
            zs.append((vr + tr, vi + ti))
            tr, ti = _cmul(k[12], k[13], cr, ci)
            self.c = (tr + jnp.broadcast_to(vr[7:8, :], (8, G)), ti + jnp.broadcast_to(vi[7:8, :], (8, G)))
        self._finish(zs, j0, j1)


def _gelu_glu(gate, up, half_scale):
    inner = gate * (0.7978845608028654 + (0.7978845608028654 * 0.044715) * (gate * gate))
    a = gate * (up * half_scale)
    return a + a * jnp.tanh(inner)


def _make_kernel(S, D, P, F):
    NF = F // TF
    Q = S // 4
    KQ = D // 4
    ND = D // 4
    KO = P // 2
    NX = S // RX
    NO = Q // RO
    R = 16

    def kernel(lre_h, lim_h, ldt_h, dsk_h, gw_h,
               x_h, bre_h, bim_h, cre_h, cim_h, wg_h, wu_h, wd_h, out_h,
               x_v, xa1, xa2, acc, hre, him, wg_v, wu_v, wd_v, bre_v, bim_v, cre_v, cim_v, cc,
               b0w, va, vb, gb, cst, carry, ost, lre_ref, lim_ref, ldt_ref, dsk_ref, gw_ref,
               sem_x, sem_b, sem_w, sem_c, sem_o, sem_v):

        def w_copies(f, slot):
            cs = pl.ds(pl.multiple_of(f * TF, TF), TF)
            rs = pl.ds(pl.multiple_of((f + 1) * G, G), G)
            return [
                pltpu.make_async_copy(bre_h.at[rs, :], bre_v.at[slot], sem_w.at[slot * 5 + 0]),
                pltpu.make_async_copy(bim_h.at[rs, :], bim_v.at[slot], sem_w.at[slot * 5 + 1]),
                pltpu.make_async_copy(wg_h.at[:, cs], wg_v.at[slot], sem_w.at[slot * 5 + 2]),
                pltpu.make_async_copy(wu_h.at[:, cs], wu_v.at[slot], sem_w.at[slot * 5 + 3]),
                pltpu.make_async_copy(wd_h.at[cs, :], wd_v.at[slot], sem_w.at[slot * 5 + 4]),
            ]

        def row0(n, size):
            return n * size if isinstance(n, int) else pl.multiple_of(n * size, size)

        def x_copy(n):
            r0 = row0(n, RX)
            return pltpu.make_async_copy(x_h.at[0, pl.ds(r0, RX), :], x_v.at[pl.ds(r0, RX), :], sem_x.at[n % 2])

        cb0r = pltpu.make_async_copy(bre_h.at[0:G, :], bre_v.at[1], sem_b.at[0])
        cb0i = pltpu.make_async_copy(bim_h.at[0:G, :], bim_v.at[1], sem_b.at[1])
        vec_copies = [pltpu.make_async_copy(src, dst, sem_v.at[i]) for i, (src, dst) in enumerate(
            ((lre_h, lre_ref), (lim_h, lim_ref), (ldt_h, ldt_ref), (gw_h, gw_ref), (dsk_h, dsk_ref)))]
        for c in vec_copies:
            c.start()
        cb0r.start()
        cb0i.start()
        x_copy(0).start()
        for c in vec_copies:
            c.wait()
        x_copy(1).start()
        _setup_consts(lre_ref, lim_ref, ldt_ref, cst)
        carry[...] = jnp.zeros_like(carry)
        cb0r.wait()
        cb0i.wait()
        b0w[0] = pltpu.bitcast(bre_v[1], U32)
        b0w[1] = pltpu.bitcast(bim_v[1], U32)
        gw = gw_ref[...].astype(F32).reshape(1, D)

        def x_wait_start(n):
            x_copy(n).wait()

            @pl.when(n + 2 < NX)
            def _():
                x_copy(n + 2).start()

            @pl.when(n == NX - 3)
            def _():
                for c in w_copies(0, 0):
                    c.start()

        def gate_rows(n):
            r0 = row0(n, RX)
            for rt in range(RX // 8):
                rows = pl.ds(r0 + rt * 8, 8)
                t = None
                for lt in range(D // 128):
                    ls = slice(lt * 128, (lt + 1) * 128)
                    p = x_v[rows, ls].astype(F32) * gw[:, ls]
                    t = p if t is None else t + p
                g = jax.nn.sigmoid(jnp.sum(t, axis=-1, keepdims=True))
                gb[rows, :] = jnp.broadcast_to(g, (8, 128))

        def in_proj0(n, vbuf):
            lhs = x_v[pl.ds(row0(n, RX), RX), :]
            for ri in range(2):
                vbuf[ri] = _dot(lhs, _as_bf16(b0w[ri]), NT)

        def scan0(n, vbuf, parallel=False):
            r0 = row0(n, RX)

            def store(a, b, hr, hi):
                hre[pl.ds(r0 + a, b - a), 0:G] = hr
                him[pl.ds(r0 + a, b - a), 0:G] = hi

            sc = _Scan(lambda a, b: vbuf[0, a:b, :], lambda a, b: vbuf[1, a:b, :], cst.at[0],
                       lambda a, b: gb[pl.ds(r0 + a, b - a), :], store)
            cr, ci = carry[0], carry[1]
            if parallel:
                sc.c = (jnp.broadcast_to(cr[7:8, :], (8, G)), jnp.broadcast_to(ci[7:8, :], (8, G)))
                sc.piece_parallel(0, RX // 8)
            else:
                sc.c = (cr, ci)
                for j in range(0, RX // 8, 8):
                    sc.piece(j, j + 8)
                carry[0] = sc.c[0]
                carry[1] = sc.c[1]

        def pro_body(m, _):
            x_wait_start(2 * m + 1)
            in_proj0(2 * m + 1, vb)
            scan0(2 * m, va)
            gate_rows(2 * m + 1)
            x_wait_start(2 * m + 2)
            in_proj0(2 * m + 2, va)
            scan0(2 * m + 1, vb)
            gate_rows(2 * m + 2)
            return 0

        x_wait_start(0)
        in_proj0(0, va)
        gate_rows(0)
        lax.fori_loop(0, NX // 2 - 1, pro_body, 0)
        x_wait_start(NX - 1)
        in_proj0(NX - 1, vb)
        scan0(NX - 2, va)
        gate_rows(NX - 1)
        scan0(NX - 1, vb, parallel=True)

        def xc2_body(n, _):
            r0, r0h = row0(n, 16), row0(n, 8)
            for lt in range(KQ // 128):
                def raw_x(q, k):
                    c0 = k * KQ + lt * 128
                    return _split(x_v[pl.ds(q * Q + r0, 16), c0:c0 + 128])
                sd = _Side(raw_x, 2, A_FORM)
                for p in PATHS2:
                    if not _is_raw(p):
                        xa2[7 * p[0] + p[1], pl.ds(r0h, 8), lt * 128:(lt + 1) * 128] = sd.leaf(p).pack()
            return 0

        def xc1_body(n, _):
            r0, r0h = row0(n, 32), row0(n, 16)
            for rt in range(2):
                for lt in range(D // 2 // 128):
                    def raw_x(hf, k):
                        c0 = k * (D // 2) + lt * 128
                        return _split(x_v[pl.ds(hf * 2 * Q + r0 + rt * 16, 16), c0:c0 + 128])
                    sd = _Side(raw_x, 1, A_FORM)
                    for i in range(7):
                        if not _is_raw((i,)):
                            xa1[i, pl.ds(r0h + rt * 8, 8), lt * 128:(lt + 1) * 128] = sd.leaf((i,)).pack()
            return 0

        lax.fori_loop(0, Q // 16, xc2_body, 0)
        lax.fori_loop(0, 2 * Q // 32, xc1_body, 0)

        def xa1_op(i):
            if not _is_raw((i,)):
                return _as_bf16(xa1[i])
            a, b = _raw_pos((i,))
            return x_v[a * 2 * Q:(a + 1) * 2 * Q, b * 2 * KQ:(b + 1) * 2 * KQ]

        def xa2_op(p):
            if not _is_raw(p):
                return _as_bf16(xa2[7 * p[0] + p[1]])
            a, b = _raw_pos(p)
            return x_v[a * Q:(a + 1) * Q, b * KQ:(b + 1) * KQ]

        ccr = pltpu.make_async_copy(cre_h, cre_v, sem_c.at[0])
        cci = pltpu.make_async_copy(cim_h, cim_v, sem_c.at[1])

        def body(f, _):
            slot = f % 2

            @pl.when(f < NF - 1)
            def _():
                for c in w_copies(f + 1, 1 - slot):
                    c.start()

            @pl.when(f == NF - 1)
            def _():
                ccr.start()
                cci.start()

            for c in w_copies(f, slot):
                c.wait()

            K2 = D // 2

            def raw_b(i, j):
                src = bre_v if j == 0 else bim_v
                return src[slot, :, i * K2:(i + 1) * K2].astype(F32)

            sb = _Side(raw_b, 1, B_FORM)
            ipp = {(i,): _dot(xa1_op(i), sb.leaf((i,)).astype(BF16), NT) for i in IP_ORDER}
            v = _Out(lambda p: ipp[p], 1)

            def raw_w(i, j):
                rows, cols = slice(i * KQ, (i + 1) * KQ), slice(j * 128, (j + 1) * 128)
                return jnp.concatenate([wg_v[slot, rows, cols].astype(F32), wu_v[slot, rows, cols].astype(F32)], 1)

            sw = _Side(raw_w, 2, B_FORM)
            gu = {}
            outs = [_Out((lambda p, t=t: gu[p][t * R:(t + 1) * R]), 2) for t in range(Q // R)]
            for i in GU_ORDER[0]:
                for j in GU_ORDER[1]:
                    gu[(i, j)] = _dot(xa2_op((i, j)), sw.leaf((i, j)).astype(BF16))
                for o in outs:
                    for a in range(2):
                        for b in range(2):
                            o.node((i,), a, b)

            h = {}
            for t, o in enumerate(outs):
                for q in range(4):
                    hs = 0.5 - 0.5 * gb[q * Q + t * R:q * Q + (t + 1) * R, :]
                    for j in range(4):
                        blk = o.block(q, j)
                        h[(q, j, t)] = _gelu_glu(blk[:, :128], blk[:, 128:], hs)

            H = S // 2
            cs = pl.ds(pl.multiple_of((f + 1) * G, G), G)

            def v_rows(ri):
                return lambda a, b: (v.block(0, ri)[a:b] if b <= H else v.block(1, ri)[a - H:b - H])

            def store(a, b, hr, hi):
                hre[a:b, cs] = hr
                him[a:b, cs] = hi

            sc = _Scan(v_rows(0), v_rows(1), cst.at[f + 1], lambda a, b: gb[a:b, :], store)
            zero = jnp.minimum(jnp.abs(gu[SCAN_AFTER][0:8, 0:G]), 0.0)
            sc.c = (zero, zero)
            for j in range(0, S // 8, 8):
                sc.piece(j, j + 8)

            KD = TF // 4
            sides = [_Side((lambda q, k, t=t: h[(q, k, t)]), 2, A_FORM) for t in range(Q // R)]

            def raw_d(i, j):
                return wd_v[slot, i * KD:(i + 1) * KD, j * ND:(j + 1) * ND].astype(F32)

            sdn = _Side(raw_d, 2, B_FORM)
            for i in DN_ORDER[0]:
                for j in DN_ORDER[1]:
                    lhs = jnp.concatenate([sd.leaf((i, j)) for sd in sides], 0).astype(BF16)
                    m = _dot(lhs, sdn.leaf((i, j)).astype(BF16))
                    acc[7 * i + j] = jnp.where(f > 0, acc[7 * i + j], 0.0) + m
            return 0

        lax.fori_loop(0, NF, body, 0)

        ccr.wait()
        cci.wait()

        def cc_body(n, _):
            r0, r0h = row0(n, 16), row0(n, 8)
            for lt in range(KO // 128):
                def raw_c(k, nq):
                    src = cre_v if k < 2 else cim_v
                    c0 = (k % 2) * KO + lt * 128
                    return _split(src[pl.ds(nq * ND + r0, 16), c0:c0 + 128])
                sd = _Side(raw_c, 2, B_FORM)
                for p in PATHS2:
                    cc[7 * p[0] + p[1], pl.ds(r0h, 8), lt * 128:(lt + 1) * 128] = sd.leaf(p).pack()
            return 0

        lax.fori_loop(0, ND // 16, cc_body, 0)

        dsk = dsk_ref[...].astype(F32).reshape(1, D)

        def o_copies(r, slot):
            r0 = row0(r, RO)
            return [pltpu.make_async_copy(ost.at[slot, q], out_h.at[0, pl.ds(q * Q + r0, RO), :],
                                          sem_o.at[slot * 4 + q]) for q in range(4)]

        def obody(r, _):
            slot = r % 2
            r0 = row0(r, RO)

            @pl.when(r >= 2)
            def _():
                for c in o_copies(r - 2, slot):
                    c.wait()

            def h_block(q, k):
                src = hre if k < 2 else him
                return src[pl.ds(q * Q + r0, RO), (k % 2) * KO:(k % 2 + 1) * KO]

            sh = _Side(lambda q, k: _split(h_block(q, k)), 2, A_FORM)
            tot = {}
            for i in OP_ORDER[0]:
                for j in OP_ORDER[1]:
                    p = (i, j)
                    lhs = h_block(*_raw_pos(p)) if _is_raw(p) else _as_bf16(sh.leaf(p).pack())
                    tot[p] = acc[7 * i + j, pl.ds(r0, RO), :] + _dot(lhs, _as_bf16(cc[7 * i + j]), NT)
            for rt in range(RO // 8):
                for lt in range(ND // 128):
                    o = _Out(lambda p: tot[p][rt * 8:(rt + 1) * 8, lt * 128:(lt + 1) * 128], 2)
                    for q in range(4):
                        rows = pl.ds(q * Q + r0 + rt * 8, 8)
                        gq = gb[rows, :]
                        for nq in range(4):
                            c0 = nq * ND + lt * 128
                            skip = x_v[rows, c0:c0 + 128].astype(F32) * dsk[:, c0:c0 + 128]
                            ost[slot, q, rt * 8:(rt + 1) * 8, c0:c0 + 128] = o.block(q, nq) + skip * gq
            for c in o_copies(r, slot):
                c.start()
            return 0

        lax.fori_loop(0, NO, obody, 0)
        for r in (NO - 2, NO - 1):
            for c in o_copies(r, r % 2):
                c.wait()

    return kernel


@jax.jit
def pallas_gated_mix__ssm_conv_s5__glu_gated_geglu__prompt_kernel(
    A_x: jax.Array,
    A_Lambda_re: jax.Array,
    A_Lambda_im: jax.Array,
    A_B_re: jax.Array,
    A_B_im: jax.Array,
    A_C_re: jax.Array,
    A_C_im: jax.Array,
    A_log_dt: jax.Array,
    A_Dskip: jax.Array,
    B_x: jax.Array,
    B_w_gate: jax.Array,
    B_w_up: jax.Array,
    B_w_down: jax.Array,
    gate_w: jax.Array,
):
    del B_x
    nb, S, D = A_x.shape
    P = A_Lambda_re.shape[0]
    F = B_w_gate.shape[1]
    assert nb == 1 and P == D and P // G == F // TF + 1 and F % TF == 0
    assert D % 1024 == 0 and S % 2048 == 0 and (S // RX) % 2 == 0 and S // RX >= 4
    Q = S // 4

    hbm = pl.BlockSpec(memory_space=pl.ANY)
    return pl.pallas_call(
        _make_kernel(S, D, P, F),
        in_specs=[hbm] * 13,
        out_specs=hbm,
        out_shape=jax.ShapeDtypeStruct((1, S, D), F32),
        scratch_shapes=[
            pltpu.VMEM((S, D), BF16),
            pltpu.VMEM((7, S // 4, D // 2), U32),
            pltpu.VMEM((49, Q // 2, D // 4), U32),
            pltpu.VMEM((49, Q, D // 4), F32),
            pltpu.VMEM((S, P), BF16),
            pltpu.VMEM((S, P), BF16),
            pltpu.VMEM((2, D, TF), BF16),
            pltpu.VMEM((2, D, TF), BF16),
            pltpu.VMEM((2, TF, D), BF16),
            pltpu.VMEM((2, G, D), BF16),
            pltpu.VMEM((2, G, D), BF16),
            pltpu.VMEM((D, P), BF16),
            pltpu.VMEM((D, P), BF16),
            pltpu.VMEM((49, D // 8, P // 2), U32),
            pltpu.VMEM((2, G // 2, D), U32),
            pltpu.VMEM((2, RX, G), F32),
            pltpu.VMEM((2, RX, G), F32),
            pltpu.VMEM((S, 128), F32),
            pltpu.VMEM((P // G, NCONST, 8, G), F32),
            pltpu.VMEM((2, 8, G), F32),
            pltpu.VMEM((2, 4, RO, D), F32),
            pltpu.VMEM((P,), A_Lambda_re.dtype),
            pltpu.VMEM((P,), A_Lambda_im.dtype),
            pltpu.VMEM((P,), A_log_dt.dtype),
            pltpu.VMEM((D,), A_Dskip.dtype),
            pltpu.VMEM((D,), gate_w.dtype),
            pltpu.SemaphoreType.DMA((2,)),
            pltpu.SemaphoreType.DMA((2,)),
            pltpu.SemaphoreType.DMA((10,)),
            pltpu.SemaphoreType.DMA((2,)),
            pltpu.SemaphoreType.DMA((8,)),
            pltpu.SemaphoreType.DMA((5,)),
        ],
        compiler_params=pltpu.CompilerParams(vmem_limit_bytes=126 * 1024 * 1024),
    )(A_Lambda_re, A_Lambda_im, A_log_dt, A_Dskip, gate_w,
      A_x, A_B_re, A_B_im, A_C_re, A_C_im, B_w_gate, B_w_up, B_w_down)
```

```python
import jax
import jax.numpy as jnp
from jax import lax
import jax.experimental.pallas as pl
import jax.experimental.pallas.tpu as pltpu

F32 = jnp.float32
BF16 = jnp.bfloat16
U32 = jnp.uint32
NN = (((1,), (0,)), ((), ()))
NT = (((1,), (1,)), ((), ()))

A_FORM = [((1, 0), (1, 3)), ((1, 2), (1, 3)), ((1, 0),), ((1, 3),), ((1, 0), (1, 1)), ((1, 2), (-1, 0)), ((1, 1), (-1, 3))]
B_FORM = [((1, 0), (1, 3)), ((1, 0),), ((1, 1), (-1, 3)), ((1, 2), (-1, 0)), ((1, 3),), ((1, 0), (1, 1)), ((1, 2), (1, 3))]
C_FORM = [((1, 0), (1, 3), (-1, 4), (1, 6)), ((1, 2), (1, 4)), ((1, 1), (1, 3)), ((1, 0), (-1, 1), (1, 2), (1, 5))]

TF = 512
G = 128
RX = 256
RO = 64
NCONST = 14

IP_ORDER = (1, 0, 6, 3, 4, 2, 5)
GU_ORDER = ((2, 0, 5, 1, 3, 4, 6), (1, 0, 3, 4, 2, 5, 6))
DN_ORDER = ((0, 6, 2, 4, 1, 3, 5), (4, 6, 3, 1, 0, 5, 2))
OP_ORDER = ((2, 3, 4, 1, 0, 5, 6), (2, 3, 5, 4, 1, 0, 6))
SCAN_AFTER = (2, 6)


def _dot(a, b, dn=NN):
    return lax.dot_general(a, b, dn, preferred_element_type=F32)


def _pack(v):
    return pltpu.bitcast(v.astype(BF16), U32)


def _split(tile):
    return tile.astype(F32)


def _as_bf16(words):
    return pltpu.bitcast(words, BF16)


def _lin(form, get):
    out = None
    for sgn, idx in form:
        t = get(idx)
        out = t if out is None else (out + t if sgn > 0 else out - t)
    return out


class _Side:
    def __init__(self, raw, lvl, form):
        self.raw, self.lvl, self.form, self.memo = raw, lvl, form, {}

    def node(self, path, i, j):
        key = (path, i, j)
        if key not in self.memo:
            if not path:
                self.memo[key] = self.raw(i, j)
            else:
                n = 2 ** (self.lvl - len(path))
                self.memo[key] = _lin(self.form[path[-1]],
                                      lambda q: self.node(path[:-1], (q // 2) * n + i, (q % 2) * n + j))
        return self.memo[key]

    def leaf(self, path):
        return self.node(tuple(path), 0, 0)


class _Out:
    def __init__(self, prod, lvl):
        self.prod, self.lvl, self.memo = prod, lvl, {}

    def node(self, path, i, j):
        key = (path, i, j)
        if key not in self.memo:
            if len(path) == self.lvl:
                self.memo[key] = self.prod(path)
            else:
                n = 2 ** (self.lvl - len(path) - 1)
                self.memo[key] = _lin(C_FORM[(i // n) * 2 + (j // n)],
                                      lambda m: self.node(path + (m,), i % n, j % n))
        return self.memo[key]

    def block(self, i, j):
        return self.node((), i, j)


PATHS2 = [(i, j) for i in range(7) for j in range(7)]


def _is_raw(path):
    return all(len(A_FORM[a]) == 1 for a in path)


def _raw_pos(path):
    i = j = 0
    for a in path:
        q = A_FORM[a][0][1]
        i, j = 2 * i + q // 2, 2 * j + q % 2
    return i, j


def _cmul(ar, ai, br, bi):
    return ar * br - ai * bi, ar * bi + ai * br


def _cdiv(ar, ai, br, bi):
    big = jnp.abs(br) >= jnp.abs(bi)
    p = jnp.where(big, bi, br)
    q = jnp.where(big, br, bi)
    r = p / q
    den = q + p * r
    u = jnp.where(big, ar, ai)
    v = jnp.where(big, ai, ar)
    re = (u + v * r) / den
    im = (v - u * r) / den
    return re, jnp.where(big, im, -im)


def _setup_consts(lre_ref, lim_ref, ldt_ref, cst):
    P = lre_ref.shape[0]

    def ld(r):
        return jnp.broadcast_to(r[...].astype(F32).reshape(1, P), (8, P))

    lre, lim, ldt = ld(lre_ref), ld(lim_ref), ld(ldt_ref)
    dt = jnp.exp(ldt).astype(ldt_ref.dtype).astype(F32)
    s = lax.broadcasted_iota(jnp.int32, (8, P), 0)
    k = (s + 1).astype(F32)
    zr = dt * lre
    zi = dt * lim
    mag = jnp.exp(zr * k)
    pr = mag * jnp.cos(zi * k)
    pi = mag * jnp.sin(zi * k)

    def row(a, r):
        return jnp.broadcast_to(a[r:r + 1, :], (8, P))

    cr, ci = _cdiv(row(pr, 0) - 1.0, row(pi, 0), lre, lim)
    vals = [jnp.where(s == 0, row(pr, 0), 0.0), jnp.where(s == 0, row(pi, 0), 0.0), 2.0 * cr, 2.0 * ci]
    for kk in (1, 2, 4):
        vals.append(jnp.where(s >= kk, row(pr, kk - 1), 0.0))
        vals.append(jnp.where(s >= kk, row(pi, kk - 1), 0.0))
    vals += [pr, pi, row(pr, 7), row(pi, 7)]
    for i, v in enumerate(vals):
        for c in range(P // G):
            cst[c, i] = v[:, c * G:(c + 1) * G]


class _Scan:
    def __init__(self, vr_fn, vi_fn, cst, g_fn, store):
        self.vr_fn, self.vi_fn, self.g_fn, self.store = vr_fn, vi_fn, g_fn, store
        self.k = [cst[i] for i in range(NCONST)]
        self.c = None

    def _prefix(self, vr, vi):
        k = self.k
        for a, kk in enumerate((1, 2, 4)):
            tr, ti = _cmul(k[4 + 2 * a], k[5 + 2 * a], pltpu.roll(vr, kk, 0), pltpu.roll(vi, kk, 0))
            vr, vi = vr + tr, vi + ti
        return vr, vi

    def _finish(self, zs, j0, j1):
        k = self.k
        gs_all = self.g_fn(j0 * 8, j1 * 8)
        hr, hi = [], []
        for j, (zr, zi) in enumerate(zs):
            gs = gs_all[j * 8:(j + 1) * 8]
            zr, zi = zr * gs, zi * gs
            hr.append(k[2] * zr - k[3] * zi)
            hi.append(-(k[2] * zi + k[3] * zr))
        self.store(j0 * 8, j1 * 8, jnp.concatenate(hr, 0).astype(BF16), jnp.concatenate(hi, 0).astype(BF16))

    def piece(self, j0, j1):
        k = self.k
        vr_all, vi_all = self.vr_fn(j0 * 8, j1 * 8), self.vi_fn(j0 * 8, j1 * 8)
        zs = []
        for j in range(j1 - j0):
            vr, vi = vr_all[j * 8:(j + 1) * 8], vi_all[j * 8:(j + 1) * 8]
            if self.c is not None:
                tr, ti = _cmul(k[0], k[1], pltpu.roll(self.c[0], 1, 0), pltpu.roll(self.c[1], 1, 0))
                vr, vi = vr + tr, vi + ti
            self.c = self._prefix(vr, vi)
            zs.append(self.c)
        self._finish(zs, j0, j1)

    def piece_parallel(self, j0, j1):
        k = self.k
        vr_all, vi_all = self.vr_fn(j0 * 8, j1 * 8), self.vi_fn(j0 * 8, j1 * 8)
        zs = []
        for j in range(j1 - j0):
            vr, vi = self._prefix(vr_all[j * 8:(j + 1) * 8], vi_all[j * 8:(j + 1) * 8])
            cr, ci = self.c
            tr, ti = _cmul(k[10], k[11], cr, ci)
            zs.append((vr + tr, vi + ti))
            tr, ti = _cmul(k[12], k[13], cr, ci)
            self.c = (tr + jnp.broadcast_to(vr[7:8, :], (8, G)), ti + jnp.broadcast_to(vi[7:8, :], (8, G)))
        self._finish(zs, j0, j1)


def _gelu_glu(gate, up, half_scale):
    inner = gate * (0.7978845608028654 + (0.7978845608028654 * 0.044715) * (gate * gate))
    a = gate * (up * half_scale)
    return a + a * jnp.tanh(inner)


def _make_kernel(S, D, P, F):
    NF = F // TF
    Q = S // 4
    KQ = D // 4
    ND = D // 4
    KO = P // 2
    NX = S // RX
    NO = Q // RO
    R = 16

    def kernel(lre_h, lim_h, ldt_h, dsk_h, gw_h,
               x_h, bre_h, bim_h, cre_h, cim_h, wg_h, wu_h, wd_h, out_h,
               x_v, xa1, xa2, acc, hre, him, wg_v, wu_v, wd_v, bre_v, bim_v, cre_v, cim_v, cc,
               b0w, va, vb, gb, cst, carry, ost, lre_ref, lim_ref, ldt_ref, dsk_ref, gw_ref,
               sem_x, sem_b, sem_w, sem_c, sem_o, sem_v):

        def w_copies(f, slot):
            cs = pl.ds(pl.multiple_of(f * TF, TF), TF)
            rs = pl.ds(pl.multiple_of((f + 1) * G, G), G)
            return [
                pltpu.make_async_copy(bre_h.at[rs, :], bre_v.at[slot], sem_w.at[slot * 5 + 0]),
                pltpu.make_async_copy(bim_h.at[rs, :], bim_v.at[slot], sem_w.at[slot * 5 + 1]),
                pltpu.make_async_copy(wg_h.at[:, cs], wg_v.at[slot], sem_w.at[slot * 5 + 2]),
                pltpu.make_async_copy(wu_h.at[:, cs], wu_v.at[slot], sem_w.at[slot * 5 + 3]),
                pltpu.make_async_copy(wd_h.at[cs, :], wd_v.at[slot], sem_w.at[slot * 5 + 4]),
            ]

        def row0(n, size):
            return n * size if isinstance(n, int) else pl.multiple_of(n * size, size)

        def x_copy(n):
            r0 = row0(n, RX)
            return pltpu.make_async_copy(x_h.at[0, pl.ds(r0, RX), :], x_v.at[pl.ds(r0, RX), :], sem_x.at[n % 2])

        cb0r = pltpu.make_async_copy(bre_h.at[0:G, :], bre_v.at[1], sem_b.at[0])
        cb0i = pltpu.make_async_copy(bim_h.at[0:G, :], bim_v.at[1], sem_b.at[1])
        vec_copies = [pltpu.make_async_copy(src, dst, sem_v.at[i]) for i, (src, dst) in enumerate(
            ((lre_h, lre_ref), (lim_h, lim_ref), (ldt_h, ldt_ref), (gw_h, gw_ref), (dsk_h, dsk_ref)))]
        for c in vec_copies:
            c.start()
        cb0r.start()
        cb0i.start()
        x_copy(0).start()
        for c in vec_copies:
            c.wait()
        x_copy(1).start()
        _setup_consts(lre_ref, lim_ref, ldt_ref, cst)
        carry[...] = jnp.zeros_like(carry)
        cb0r.wait()
        cb0i.wait()
        b0w[0] = pltpu.bitcast(bre_v[1], U32)
        b0w[1] = pltpu.bitcast(bim_v[1], U32)
        gw = gw_ref[...].astype(F32).reshape(1, D)

        def x_wait_start(n):
            x_copy(n).wait()

            @pl.when(n + 2 < NX)
            def _():
                x_copy(n + 2).start()

            @pl.when(n == NX - 3)
            def _():
                for c in w_copies(0, 0):
                    c.start()

        def gate_rows(n):
            r0 = row0(n, RX)
            for rt in range(RX // 8):
                rows = pl.ds(r0 + rt * 8, 8)
                t = None
                for lt in range(D // 128):
                    ls = slice(lt * 128, (lt + 1) * 128)
                    p = x_v[rows, ls].astype(F32) * gw[:, ls]
                    t = p if t is None else t + p
                g = jax.nn.sigmoid(jnp.sum(t, axis=-1, keepdims=True))
                gb[rows, :] = jnp.broadcast_to(g, (8, 128))

        def in_proj0(n, vbuf):
            lhs = x_v[pl.ds(row0(n, RX), RX), :]
            for ri in range(2):
                vbuf[ri] = _dot(lhs, _as_bf16(b0w[ri]), NT)

        def scan0(n, vbuf, parallel=False):
            r0 = row0(n, RX)

            def store(a, b, hr, hi):
                hre[pl.ds(r0 + a, b - a), 0:G] = hr
                him[pl.ds(r0 + a, b - a), 0:G] = hi

            sc = _Scan(lambda a, b: vbuf[0, a:b, :], lambda a, b: vbuf[1, a:b, :], cst.at[0],
                       lambda a, b: gb[pl.ds(r0 + a, b - a), :], store)
            cr, ci = carry[0], carry[1]
            if parallel:
                sc.c = (jnp.broadcast_to(cr[7:8, :], (8, G)), jnp.broadcast_to(ci[7:8, :], (8, G)))
                sc.piece_parallel(0, RX // 8)
            else:
                sc.c = (cr, ci)
                for j in range(0, RX // 8, 8):
                    sc.piece(j, j + 8)
                carry[0] = sc.c[0]
                carry[1] = sc.c[1]

        def pro_body(m, _):
            x_wait_start(2 * m + 1)
            in_proj0(2 * m + 1, vb)
            scan0(2 * m, va)
            gate_rows(2 * m + 1)
            x_wait_start(2 * m + 2)
            in_proj0(2 * m + 2, va)
            scan0(2 * m + 1, vb)
            gate_rows(2 * m + 2)
            return 0

        x_wait_start(0)
        in_proj0(0, va)
        gate_rows(0)
        lax.fori_loop(0, NX // 2 - 1, pro_body, 0)
        x_wait_start(NX - 1)
        in_proj0(NX - 1, vb)
        scan0(NX - 2, va)
        gate_rows(NX - 1)
        scan0(NX - 1, vb, parallel=True)

        def xc2_body(n, _):
            r0, r0h = row0(n, 16), row0(n, 8)
            for lt in range(KQ // 128):
                def raw_x(q, k):
                    c0 = k * KQ + lt * 128
                    return _split(x_v[pl.ds(q * Q + r0, 16), c0:c0 + 128])
                sd = _Side(raw_x, 2, A_FORM)
                for p in PATHS2:
                    if not _is_raw(p):
                        xa2[7 * p[0] + p[1], pl.ds(r0h, 8), lt * 128:(lt + 1) * 128] = _pack(sd.leaf(p))
            return 0

        def xc1_body(n, _):
            r0, r0h = row0(n, 32), row0(n, 16)
            for rt in range(2):
                for lt in range(D // 2 // 128):
                    def raw_x(hf, k):
                        c0 = k * (D // 2) + lt * 128
                        return _split(x_v[pl.ds(hf * 2 * Q + r0 + rt * 16, 16), c0:c0 + 128])
                    sd = _Side(raw_x, 1, A_FORM)
                    for i in range(7):
                        if not _is_raw((i,)):
                            xa1[i, pl.ds(r0h + rt * 8, 8), lt * 128:(lt + 1) * 128] = _pack(sd.leaf((i,)))
            return 0

        lax.fori_loop(0, Q // 16, xc2_body, 0)
        lax.fori_loop(0, 2 * Q // 32, xc1_body, 0)

        def xa1_op(i):
            if not _is_raw((i,)):
                return _as_bf16(xa1[i])
            a, b = _raw_pos((i,))
            return x_v[a * 2 * Q:(a + 1) * 2 * Q, b * 2 * KQ:(b + 1) * 2 * KQ]

        def xa2_op(p):
            if not _is_raw(p):
                return _as_bf16(xa2[7 * p[0] + p[1]])
            a, b = _raw_pos(p)
            return x_v[a * Q:(a + 1) * Q, b * KQ:(b + 1) * KQ]

        ccr = pltpu.make_async_copy(cre_h, cre_v, sem_c.at[0])
        cci = pltpu.make_async_copy(cim_h, cim_v, sem_c.at[1])

        def body(f, _):
            slot = f % 2

            @pl.when(f < NF - 1)
            def _():
                for c in w_copies(f + 1, 1 - slot):
                    c.start()

            @pl.when(f == NF - 1)
            def _():
                ccr.start()
                cci.start()

            for c in w_copies(f, slot):
                c.wait()

            K2 = D // 2

            def raw_b(i, j):
                src = bre_v if j == 0 else bim_v
                return src[slot, :, i * K2:(i + 1) * K2].astype(F32)

            sb = _Side(raw_b, 1, B_FORM)
            ipp = {(i,): _dot(xa1_op(i), sb.leaf((i,)).astype(BF16), NT) for i in IP_ORDER}
            v = _Out(lambda p: ipp[p], 1)

            def raw_w(i, j):
                rows, cols = slice(i * KQ, (i + 1) * KQ), slice(j * 128, (j + 1) * 128)
                return jnp.concatenate([wg_v[slot, rows, cols].astype(F32), wu_v[slot, rows, cols].astype(F32)], 1)

            sw = _Side(raw_w, 2, B_FORM)
            gu = {}
            outs = [_Out((lambda p, t=t: gu[p][t * R:(t + 1) * R]), 2) for t in range(Q // R)]
            for i in GU_ORDER[0]:
                for j in GU_ORDER[1]:
                    gu[(i, j)] = _dot(xa2_op((i, j)), sw.leaf((i, j)).astype(BF16))
                for o in outs:
                    for a in range(2):
                        for b in range(2):
                            o.node((i,), a, b)

            h = {}
            for t, o in enumerate(outs):
                for q in range(4):
                    hs = 0.5 - 0.5 * gb[q * Q + t * R:q * Q + (t + 1) * R, :]
                    for j in range(4):
                        blk = o.block(q, j)
                        h[(q, j, t)] = _gelu_glu(blk[:, :128], blk[:, 128:], hs)

            H = S // 2
            cs = pl.ds(pl.multiple_of((f + 1) * G, G), G)

            def v_rows(ri):
                return lambda a, b: (v.block(0, ri)[a:b] if b <= H else v.block(1, ri)[a - H:b - H])

            def store(a, b, hr, hi):
                hre[a:b, cs] = hr
                him[a:b, cs] = hi

            sc = _Scan(v_rows(0), v_rows(1), cst.at[f + 1], lambda a, b: gb[a:b, :], store)
            zero = jnp.minimum(jnp.abs(gu[SCAN_AFTER][0:8, 0:G]), 0.0)
            sc.c = (zero, zero)
            for j in range(0, S // 8, 8):
                sc.piece(j, j + 8)

            KD = TF // 4
            sides = [_Side((lambda q, k, t=t: h[(q, k, t)]), 2, A_FORM) for t in range(Q // R)]

            def raw_d(i, j):
                return wd_v[slot, i * KD:(i + 1) * KD, j * ND:(j + 1) * ND].astype(F32)

            sdn = _Side(raw_d, 2, B_FORM)
            for i in DN_ORDER[0]:
                for j in DN_ORDER[1]:
                    lhs = jnp.concatenate([sd.leaf((i, j)) for sd in sides], 0).astype(BF16)
                    m = _dot(lhs, sdn.leaf((i, j)).astype(BF16))
                    acc[7 * i + j] = jnp.where(f > 0, acc[7 * i + j], 0.0) + m
            return 0

        lax.fori_loop(0, NF, body, 0)

        ccr.wait()
        cci.wait()

        def cc_body(n, _):
            r0, r0h = row0(n, 16), row0(n, 8)
            for lt in range(KO // 128):
                def raw_c(k, nq):
                    src = cre_v if k < 2 else cim_v
                    c0 = (k % 2) * KO + lt * 128
                    return _split(src[pl.ds(nq * ND + r0, 16), c0:c0 + 128])
                sd = _Side(raw_c, 2, B_FORM)
                for p in PATHS2:
                    cc[7 * p[0] + p[1], pl.ds(r0h, 8), lt * 128:(lt + 1) * 128] = _pack(sd.leaf(p))
            return 0

        lax.fori_loop(0, ND // 16, cc_body, 0)

        dsk = dsk_ref[...].astype(F32).reshape(1, D)

        def o_copies(r, slot):
            r0 = row0(r, RO)
            return [pltpu.make_async_copy(ost.at[slot, q], out_h.at[0, pl.ds(q * Q + r0, RO), :],
                                          sem_o.at[slot * 4 + q]) for q in range(4)]

        def obody(r, _):
            slot = r % 2
            r0 = row0(r, RO)

            @pl.when(r >= 2)
            def _():
                for c in o_copies(r - 2, slot):
                    c.wait()

            def h_block(q, k):
                src = hre if k < 2 else him
                return src[pl.ds(q * Q + r0, RO), (k % 2) * KO:(k % 2 + 1) * KO]

            sh = _Side(lambda q, k: _split(h_block(q, k)), 2, A_FORM)
            tot = {}
            for i in OP_ORDER[0]:
                for j in OP_ORDER[1]:
                    p = (i, j)
                    lhs = h_block(*_raw_pos(p)) if _is_raw(p) else sh.leaf(p).astype(BF16)
                    tot[p] = acc[7 * i + j, pl.ds(r0, RO), :] + _dot(lhs, _as_bf16(cc[7 * i + j]), NT)
            for rt in range(RO // 8):
                for lt in range(ND // 128):
                    o = _Out(lambda p: tot[p][rt * 8:(rt + 1) * 8, lt * 128:(lt + 1) * 128], 2)
                    for q in range(4):
                        rows = pl.ds(q * Q + r0 + rt * 8, 8)
                        gq = gb[rows, :]
                        for nq in range(4):
                            c0 = nq * ND + lt * 128
                            skip = x_v[rows, c0:c0 + 128].astype(F32) * dsk[:, c0:c0 + 128]
                            ost[slot, q, rt * 8:(rt + 1) * 8, c0:c0 + 128] = o.block(q, nq) + skip * gq
            for c in o_copies(r, slot):
                c.start()
            return 0

        lax.fori_loop(0, NO, obody, 0)
        for r in (NO - 2, NO - 1):
            for c in o_copies(r, r % 2):
                c.wait()

    return kernel


@jax.jit
def pallas_gated_mix__ssm_conv_s5__glu_gated_geglu__prompt_kernel(
    A_x: jax.Array,
    A_Lambda_re: jax.Array,
    A_Lambda_im: jax.Array,
    A_B_re: jax.Array,
    A_B_im: jax.Array,
    A_C_re: jax.Array,
    A_C_im: jax.Array,
    A_log_dt: jax.Array,
    A_Dskip: jax.Array,
    B_x: jax.Array,
    B_w_gate: jax.Array,
    B_w_up: jax.Array,
    B_w_down: jax.Array,
    gate_w: jax.Array,
):
    del B_x
    nb, S, D = A_x.shape
    P = A_Lambda_re.shape[0]
    F = B_w_gate.shape[1]
    assert nb == 1 and P == D and P // G == F // TF + 1 and F % TF == 0
    assert D % 1024 == 0 and S % 2048 == 0 and (S // RX) % 2 == 0 and S // RX >= 4
    Q = S // 4

    hbm = pl.BlockSpec(memory_space=pl.ANY)
    return pl.pallas_call(
        _make_kernel(S, D, P, F),
        in_specs=[hbm] * 13,
        out_specs=hbm,
        out_shape=jax.ShapeDtypeStruct((1, S, D), F32),
        scratch_shapes=[
            pltpu.VMEM((S, D), BF16),
            pltpu.VMEM((7, S // 4, D // 2), U32),
            pltpu.VMEM((49, Q // 2, D // 4), U32),
            pltpu.VMEM((49, Q, D // 4), F32),
            pltpu.VMEM((S, P), BF16),
            pltpu.VMEM((S, P), BF16),
            pltpu.VMEM((2, D, TF), BF16),
            pltpu.VMEM((2, D, TF), BF16),
            pltpu.VMEM((2, TF, D), BF16),
            pltpu.VMEM((2, G, D), BF16),
            pltpu.VMEM((2, G, D), BF16),
            pltpu.VMEM((D, P), BF16),
            pltpu.VMEM((D, P), BF16),
            pltpu.VMEM((49, D // 8, P // 2), U32),
            pltpu.VMEM((2, G // 2, D), U32),
            pltpu.VMEM((2, RX, G), F32),
            pltpu.VMEM((2, RX, G), F32),
            pltpu.VMEM((S, 128), F32),
            pltpu.VMEM((P // G, NCONST, 8, G), F32),
            pltpu.VMEM((2, 8, G), F32),
            pltpu.VMEM((2, 4, RO, D), F32),
            pltpu.VMEM((P,), A_Lambda_re.dtype),
            pltpu.VMEM((P,), A_Lambda_im.dtype),
            pltpu.VMEM((P,), A_log_dt.dtype),
            pltpu.VMEM((D,), A_Dskip.dtype),
            pltpu.VMEM((D,), gate_w.dtype),
            pltpu.SemaphoreType.DMA((2,)),
            pltpu.SemaphoreType.DMA((2,)),
            pltpu.SemaphoreType.DMA((10,)),
            pltpu.SemaphoreType.DMA((2,)),
            pltpu.SemaphoreType.DMA((8,)),
            pltpu.SemaphoreType.DMA((5,)),
        ],
        compiler_params=pltpu.CompilerParams(vmem_limit_bytes=126 * 1024 * 1024),
    )(A_Lambda_re, A_Lambda_im, A_log_dt, A_Dskip, gate_w,
      A_x, A_B_re, A_B_im, A_C_re, A_C_im, B_w_gate, B_w_up, B_w_down)
```
